```python
import jax
import jax.numpy as jnp

def _softmax(x, axis=-1):
    return jax.nn.softmax(x, axis=axis)

def _gelu(x):
    return jax.nn.gelu(x, approximate=True)

def _silu(x):
    return jax.nn.silu(x)

def _sigmoid(x):
    return jax.nn.sigmoid(x)

def _layernorm(x, axis=-1, eps=1e-05):
    m = jnp.mean(x, axis=axis, keepdims=True)
    v = jnp.var(x, axis=axis, keepdims=True)
    return (x - m) / jnp.sqrt(v + eps)

def _scatter_add(tgt, idx, src, axis=0):
    return tgt.at[idx].add(src)

def _segment_sum(src, seg, n):
    return jax.ops.segment_sum(src, seg, n)

class _Rng:

    def __init__(self, key):
        self._k = key

    def _next(self):
        self._k, sub = jax.random.split(self._k)
        return sub

    def normal(self, shape):
        return jax.random.normal(self._next(), shape, dtype=jnp.bfloat16)

    def randint(self, lo, hi, shape):
        return jax.random.randint(self._next(), shape, lo, hi, dtype=jnp.int32)

    def uniform(self, shape, lo=0.0, hi=1.0):
        return jax.random.uniform(self._next(), shape, jnp.bfloat16, lo, hi)

    def permutation(self, n):
        return jax.random.permutation(self._next(), n)
kernel_name = 'adaLN_cond__mha_block_cached__moe_arch_mod__decode'

def setup_inputs():
    _rng = _Rng(jax.random.key(int.from_bytes(__import__("os").urandom(4), "little")))
    _w = lambda a: (lambda t: t.astype(jnp.bfloat16) if jnp.issubdtype(t.dtype, jnp.floating) else t)(jnp.asarray(a))

    def _A_setup():
        B, Sq, D = (4, 1, 448)
        H, Sk, Dh = (16, 16384, 256)
        return {'x': _w((lambda *s: _rng.normal(s) * 0.05)(B, Sq, D)), 'k_cache': _w((lambda *s: _rng.normal(s) * 0.05)(B, H, Sk, Dh)), 'v_cache': _w((lambda *s: _rng.normal(s) * 0.05)(B, H, Sk, Dh)), 'wq': _w((lambda *s: _rng.normal(s) * 0.05)(D, H * Dh) * D ** (-0.5)), 'wo': _w((lambda *s: _rng.normal(s) * 0.05)(H * Dh, D) * (H * Dh) ** (-0.5))}
    _A_in = _A_setup()

    def _B_setup():
        B, S, D, F, C = (4, 1, 448, 1792, 1)
        return {'x': _w((lambda *s: _rng.normal(s) * 0.05)(B, S, D)), 'w_r': _w((lambda *s: _rng.normal(s) * 0.05)(D)), 'w_gate': _w((lambda *s: _rng.normal(s) * 0.05)(D, F)), 'w_up': _w((lambda *s: _rng.normal(s) * 0.05)(D, F)), 'w_down': _w((lambda *s: _rng.normal(s) * 0.05)(F, D))}
    _B_in = _B_setup()
    return {'A_x': _A_in['x'], 'A_k_cache': _A_in['k_cache'], 'A_v_cache': _A_in['v_cache'], 'A_wq': _A_in['wq'], 'A_wo': _A_in['wo'], 'B_x': _B_in['x'], 'B_w_r': _B_in['w_r'], 'B_w_gate': _B_in['w_gate'], 'B_w_up': _B_in['w_up'], 'B_w_down': _B_in['w_down'], 'c': _w((lambda *s: _rng.normal(s) * 0.05)(4, 448)), 'w_mod': _w((lambda *s: _rng.normal(s) * 0.05)(448, 6 * 448) * 448 ** (-0.5))}

def reference(A_x, A_k_cache, A_v_cache, A_wq, A_wo, B_x, B_w_r, B_w_gate, B_w_up, B_w_down, c, w_mod):

    def _A_ref(x, k_cache, v_cache, wq, wo):
        B, Sq, D = x.shape
        H, Dh = (16, 256)
        q = (lambda x, *d: x.transpose(*d))((x @ wq).reshape(B, Sq, H, Dh), 0, 2, 1, 3)
        scores = jnp.einsum('bhqd,bhkd->bhqk', q, k_cache) * Dh ** (-0.5)
        p = _softmax(scores, axis=-1)
        o = jnp.einsum('bhqk,bhkd->bhqd', p, v_cache)
        return (lambda x, *d: x.transpose(*d))(o, 0, 2, 1, 3).reshape(B, Sq, H * Dh) @ wo

    def _B_ref(x, w_r, w_gate, w_up, w_down):
        B, S, D = x.shape
        C = 1
        r = x @ w_r
        idx = jnp.argsort(-r, axis=-1)[:, :C]
        idx_e = jnp.repeat(idx.reshape(B, C, 1), D, axis=2)
        x_sel = jnp.take_along_axis(x, idx_e, axis=1)
        g = _silu(x_sel @ w_gate)
        u = x_sel @ w_up
        y = g * u @ w_down
        r_sel = _sigmoid(jnp.take_along_axis(r, idx, axis=1))
        y = y * r_sel.reshape(B, C, 1)
        b_off = (jnp.arange(B) * S).reshape(B, 1)
        flat_idx = (idx + b_off).reshape(B * C)
        zero = (x * 0.0).reshape(B * S, D)
        upd = _scatter_add(zero, flat_idx, y.reshape(B * C, D), axis=0)
        return x + upd.reshape(B, S, D)
    x = A_x
    mod = (_silu(c) @ w_mod).reshape(c.shape[0], 6, 1, -1)
    sa, ca, ga, sb, cb, gb = (mod[:, 0].copy(), mod[:, 1].copy(), mod[:, 2].copy(), mod[:, 3].copy(), mod[:, 4].copy(), mod[:, 5].copy())
    h = _layernorm(x, axis=-1) * (1 + ca) + sa
    x = x + ga * _A_ref(h, A_k_cache, A_v_cache, A_wq, A_wo)
    h = _layernorm(x, axis=-1) * (1 + cb) + sb
    x = x + gb * _B_ref(h, B_w_r, B_w_gate, B_w_up, B_w_down)
    return x
```

```python
import jax
import jax.numpy as jnp
import jax.experimental.pallas as pl
import jax.experimental.pallas.tpu as pltpu

_NT = (((1,), (1,)), ((), ()))


def _layernorm(x, eps=1e-5):
    m = jnp.mean(x, axis=-1, keepdims=True)
    d = x - m
    v = jnp.mean(d * d, axis=-1, keepdims=True)
    return d * jax.lax.rsqrt(v + eps)


def _silu(x):
    return x * jax.nn.sigmoid(x)


def _make_kernel(B, H, S, Dh, D, CH, R, ROT):
    NK = S // CH
    NP = CH // (2 * R)
    f32, bf16 = jnp.float32, jnp.bfloat16

    def kernel(x_hbm, k_hbm, v_hbm, wq_hbm, wo_hbm, wr_hbm, wg_hbm, wu_hbm, wd_hbm,
               c_hbm, wmod_hbm, o_ref,
               ring, x_v, c_v, wr_v, wmod_v, wq_v, wo_v, wg_v, wu_v, wd_v,
               q_s, s_s, ring_sem, w_sem):

        def start_chunk(src, bh, j):
            b = bh % B
            h = bh // B
            for i in range(NP):
                for p in range(2):
                    piece = p * NP + (i + p * ROT) % NP
                    pltpu.make_async_copy(
                        src.at[b, h, pl.ds(pl.multiple_of(j * CH + piece * R, R), R), :],
                        ring.at[j, pl.ds(piece * R, R), :],
                        ring_sem.at[j]).start(priority=p)

        def wait_chunk(j):
            pltpu.make_async_copy(ring.at[j], ring.at[j], ring_sem.at[j]).wait()

        early = [pltpu.make_async_copy(s, d, w_sem.at[i]) for i, (s, d) in enumerate(
            [(c_hbm, c_v), (x_hbm, x_v), (wmod_hbm, wmod_v), (wq_hbm, wq_v)])]
        late = [pltpu.make_async_copy(s, d, w_sem.at[4 + i]) for i, (s, d) in enumerate(
            [(wo_hbm, wo_v), (wr_hbm, wr_v), (wg_hbm, wg_v), (wu_hbm, wu_v), (wd_hbm, wd_v)])]

        early[0].start(priority=0)
        early[1].start(priority=0)
        early[2].start(priority=0)
        early[3].start(priority=1)

        def prime(j, carry):
            start_chunk(k_hbm, 0, j)
            return carry
        jax.lax.fori_loop(0, NK, prime, 0)
        for i, cp in enumerate(late):
            cp.start(priority=i % 2)

        early[0].wait()
        early[2].wait()
        c = c_v[...].astype(f32)
        mod = jnp.dot(_silu(c).astype(bf16), wmod_v[...], preferred_element_type=f32)
        sa, ca, ga, sb, cb, gb = [mod[:, i * D:(i + 1) * D] for i in range(6)]
        early[1].wait()
        x = x_v[...].astype(f32)
        hq = _layernorm(x) * (1.0 + ca) + sa
        early[3].wait()
        q = jnp.dot(hq.astype(bf16), wq_v[...], preferred_element_type=f32)
        q = (q * (Dh ** -0.5)).astype(bf16)
        for h in range(H):
            q_s[h] = q[:, h * Dh:(h + 1) * Dh]
        late[0].wait()

        row = jax.lax.broadcasted_iota(jnp.int32, (B, Dh), 0)

        def head(bh, carry):
            o_h, attn = carry
            b = bh % B
            h = bh // B
            qh = q_s[h]

            def k_step(j, m):
                wait_chunk(j)
                s = jax.lax.dot_general(qh, ring[j], _NT, preferred_element_type=f32)
                start_chunk(v_hbm, bh, j)
                s_s[j] = s
                return jnp.maximum(m, jnp.max(s, axis=-1, keepdims=True))
            m = jax.lax.fori_loop(0, NK, k_step, jnp.full((B, 1), -jnp.inf, f32))

            def v_step(j, la):
                l, acc = la
                p = jnp.exp(s_s[j] - m)
                l = l + jnp.sum(p, axis=-1, keepdims=True)
                wait_chunk(j)
                acc = acc + jnp.dot(p.astype(bf16), ring[j], preferred_element_type=f32)

                @pl.when(bh + 1 < B * H)
                def _():
                    start_chunk(k_hbm, bh + 1, j)
                return l, acc
            l, acc = jax.lax.fori_loop(
                0, NK, v_step, (jnp.zeros((B, 1), f32), jnp.zeros((B, Dh), f32)))

            o_h = jnp.where(row == b, acc / l, o_h)

            def proj():
                w = wo_v[:, pl.ds(pl.multiple_of(h * Dh, Dh), Dh)]
                return attn + jax.lax.dot_general(o_h.astype(bf16), w, _NT, preferred_element_type=f32)
            attn = jax.lax.cond(b == B - 1, proj, lambda: attn)
            return o_h, attn

        _, attn = jax.lax.fori_loop(
            0, B * H, head, (jnp.zeros((B, Dh), f32), jnp.zeros((B, D), f32)))

        x = x + ga * attn
        h2 = _layernorm(x) * (1.0 + cb) + sb
        for cp in late[1:]:
            cp.wait()
        h2b = h2.astype(bf16)
        r = jnp.sum(h2b.astype(f32) * wr_v[...].astype(f32).reshape(1, D), axis=-1, keepdims=True)
        g = _silu(jnp.dot(h2b, wg_v[...], preferred_element_type=f32))
        u = jnp.dot(h2b, wu_v[...], preferred_element_type=f32)
        y = jax.lax.dot_general((g * u).astype(bf16), wd_v[...], _NT, preferred_element_type=f32)
        y = y * jax.nn.sigmoid(r)
        out = x + gb * (h2 + (h2 * 0.0 + y))
        o_ref[...] = out.astype(o_ref.dtype)

    return kernel


@jax.jit
def pallas_adaLN_cond__mha_block_cached__moe_arch_mod__decode_kernel(
    A_x: jax.Array,
    A_k_cache: jax.Array,
    A_v_cache: jax.Array,
    A_wq: jax.Array,
    A_wo: jax.Array,
    B_x: jax.Array,
    B_w_r: jax.Array,
    B_w_gate: jax.Array,
    B_w_up: jax.Array,
    B_w_down: jax.Array,
    c: jax.Array,
    w_mod: jax.Array,
):
    del B_x
    B, Sq, D = A_x.shape
    _, H, S, Dh = A_k_cache.shape
    assert Sq == 1
    CH, R, ROT = 2048, 64, 3
    NK = S // CH
    kernel = _make_kernel(B, H, S, Dh, D, CH, R, ROT)
    A_x = A_x.reshape(B, D)
    A_wo = A_wo.T
    B_w_down = B_w_down.T
    ins = (A_x, A_k_cache, A_v_cache, A_wq, A_wo, B_w_r, B_w_gate, B_w_up, B_w_down, c, w_mod)

    def like(a):
        return pltpu.VMEM(a.shape, a.dtype)

    return pl.pallas_call(
        kernel,
        out_shape=jax.ShapeDtypeStruct(A_x.shape, A_x.dtype),
        in_specs=[pl.BlockSpec(memory_space=pltpu.HBM)] * len(ins),
        out_specs=pl.BlockSpec(memory_space=pltpu.VMEM),
        scratch_shapes=[
            pltpu.VMEM((NK, CH, Dh), A_k_cache.dtype),
            like(A_x), like(c), like(B_w_r), like(w_mod), like(A_wq), like(A_wo),
            like(B_w_gate), like(B_w_up), like(B_w_down),
            pltpu.VMEM((H, B, Dh), jnp.bfloat16),
            pltpu.VMEM((NK, B, CH), jnp.float32),
            pltpu.SemaphoreType.DMA((NK,)),
            pltpu.SemaphoreType.DMA((9,)),
        ],
        compiler_params=pltpu.CompilerParams(vmem_limit_bytes=100 * 1024 * 1024),
    )(*ins).reshape(B, Sq, D)
```

```python
import jax
import jax.numpy as jnp
import jax.experimental.pallas as pl
import jax.experimental.pallas.tpu as pltpu

_CFG = (4096, 64, 8, 0)
_NT = (((1,), (1,)), ((), ()))


def _layernorm(x, eps=1e-5):
    m = jnp.mean(x, axis=-1, keepdims=True)
    d = x - m
    v = jnp.mean(d * d, axis=-1, keepdims=True)
    return d * jax.lax.rsqrt(v + eps)


def _silu(x):
    return x * jax.nn.sigmoid(x)


def _make_kernel(B, H, S, Dh, D, CH, R, G, ROT):
    NK = S // CH
    NP = CH // (G * R)
    f32, bf16 = jnp.float32, jnp.bfloat16

    def kernel(x_hbm, k_hbm, v_hbm, wq_hbm, wo_hbm, wr_hbm, wg_hbm, wu_hbm, wd_hbm,
               c_hbm, wmod_hbm, o_ref,
               ring, x_v, c_v, wr_v, wmod_v, wq_v, wo_v, wg_v, wu_v, wd_v,
               q_s, s_s, ring_sem, w_sem):

        def start_chunk(src, bh, j):
            b = bh % B
            h = bh // B
            for i in range(NP):
                for g in range(G):
                    piece = g * NP + (i + g * ROT) % NP
                    pltpu.make_async_copy(
                        src.at[b, h, pl.ds(pl.multiple_of(j * CH + piece * R, R), R), :],
                        ring.at[j, pl.ds(piece * R, R), :],
                        ring_sem.at[j]).start(priority=g % 2)

        def wait_chunk(j):
            pltpu.make_async_copy(ring.at[j], ring.at[j], ring_sem.at[j]).wait()

        early = [pltpu.make_async_copy(s, d, w_sem.at[i]) for i, (s, d) in enumerate(
            [(c_hbm, c_v), (x_hbm, x_v), (wmod_hbm, wmod_v), (wq_hbm, wq_v)])]
        late = [pltpu.make_async_copy(s, d, w_sem.at[4 + i]) for i, (s, d) in enumerate(
            [(wo_hbm, wo_v), (wr_hbm, wr_v), (wg_hbm, wg_v), (wu_hbm, wu_v), (wd_hbm, wd_v)])]

        early[0].start(priority=0)
        early[1].start(priority=0)
        early[2].start(priority=0)
        early[3].start(priority=1)

        def prime(j, carry):
            start_chunk(k_hbm, 0, j)
            return carry
        jax.lax.fori_loop(0, NK, prime, 0)
        for i, cp in enumerate(late):
            cp.start(priority=i % 2)

        early[0].wait()
        early[2].wait()
        c = c_v[...].astype(f32)
        mod = jnp.dot(_silu(c).astype(bf16), wmod_v[...], preferred_element_type=f32)
        sa, ca, ga, sb, cb, gb = [mod[:, i * D:(i + 1) * D] for i in range(6)]
        early[1].wait()
        x = x_v[...].astype(f32)
        hq = _layernorm(x) * (1.0 + ca) + sa
        early[3].wait()
        q = jnp.dot(hq.astype(bf16), wq_v[...], preferred_element_type=f32)
        q = (q * (Dh ** -0.5)).astype(bf16)
        for h in range(H):
            q_s[h] = q[:, h * Dh:(h + 1) * Dh]
        late[0].wait()

        row = jax.lax.broadcasted_iota(jnp.int32, (B, Dh), 0)

        def head(bh, carry):
            o_h, attn = carry
            b = bh % B
            h = bh // B
            qh = q_s[h]

            def k_step(j, m):
                wait_chunk(j)
                s = jax.lax.dot_general(qh, ring[j], _NT, preferred_element_type=f32)
                start_chunk(v_hbm, bh, j)
                s_s[j] = s
                return jnp.maximum(m, jnp.max(s, axis=-1, keepdims=True))
            m = jax.lax.fori_loop(0, NK, k_step, jnp.full((B, 1), -jnp.inf, f32))

            def v_step(j, la):
                l, acc = la
                p = jnp.exp(s_s[j] - m)
                l = l + jnp.sum(p, axis=-1, keepdims=True)
                wait_chunk(j)
                acc = acc + jnp.dot(p.astype(bf16), ring[j], preferred_element_type=f32)

                @pl.when(bh + 1 < B * H)
                def _():
                    start_chunk(k_hbm, bh + 1, j)
                return l, acc
            l, acc = jax.lax.fori_loop(
                0, NK, v_step, (jnp.zeros((B, 1), f32), jnp.zeros((B, Dh), f32)))

            o_h = jnp.where(row == b, acc / l, o_h)

            def proj():
                w = wo_v[:, pl.ds(pl.multiple_of(h * Dh, Dh), Dh)]
                return attn + jax.lax.dot_general(o_h.astype(bf16), w, _NT, preferred_element_type=f32)
            attn = jax.lax.cond(b == B - 1, proj, lambda: attn)
            return o_h, attn

        _, attn = jax.lax.fori_loop(
            0, B * H, head, (jnp.zeros((B, Dh), f32), jnp.zeros((B, D), f32)))

        x = x + ga * attn
        h2 = _layernorm(x) * (1.0 + cb) + sb
        for cp in late[1:]:
            cp.wait()
        h2b = h2.astype(bf16)
        r = jnp.sum(h2b.astype(f32) * wr_v[...].astype(f32).reshape(1, D), axis=-1, keepdims=True)
        g = _silu(jnp.dot(h2b, wg_v[...], preferred_element_type=f32))
        u = jnp.dot(h2b, wu_v[...], preferred_element_type=f32)
        y = jax.lax.dot_general((g * u).astype(bf16), wd_v[...], _NT, preferred_element_type=f32)
        y = y * jax.nn.sigmoid(r)
        out = x + gb * (h2 + (h2 * 0.0 + y))
        o_ref[...] = out.astype(o_ref.dtype)

    return kernel


@jax.jit
def pallas_adaLN_cond__mha_block_cached__moe_arch_mod__decode_kernel(
    A_x: jax.Array,
    A_k_cache: jax.Array,
    A_v_cache: jax.Array,
    A_wq: jax.Array,
    A_wo: jax.Array,
    B_x: jax.Array,
    B_w_r: jax.Array,
    B_w_gate: jax.Array,
    B_w_up: jax.Array,
    B_w_down: jax.Array,
    c: jax.Array,
    w_mod: jax.Array,
):
    del B_x
    B, Sq, D = A_x.shape
    _, H, S, Dh = A_k_cache.shape
    assert Sq == 1
    CH, R, G, ROT = _CFG
    NK = S // CH
    kernel = _make_kernel(B, H, S, Dh, D, CH, R, G, ROT)
    A_x = A_x.reshape(B, D)
    A_wo = A_wo.T
    B_w_down = B_w_down.T
    ins = (A_x, A_k_cache, A_v_cache, A_wq, A_wo, B_w_r, B_w_gate, B_w_up, B_w_down, c, w_mod)

    def like(a):
        return pltpu.VMEM(a.shape, a.dtype)

    return pl.pallas_call(
        kernel,
        out_shape=jax.ShapeDtypeStruct(A_x.shape, A_x.dtype),
        in_specs=[pl.BlockSpec(memory_space=pltpu.HBM)] * len(ins),
        out_specs=pl.BlockSpec(memory_space=pltpu.VMEM),
        scratch_shapes=[
            pltpu.VMEM((NK, CH, Dh), A_k_cache.dtype),
            like(A_x), like(c), like(B_w_r), like(w_mod), like(A_wq), like(A_wo),
            like(B_w_gate), like(B_w_up), like(B_w_down),
            pltpu.VMEM((H, B, Dh), jnp.bfloat16),
            pltpu.VMEM((NK, B, CH), jnp.float32),
            pltpu.SemaphoreType.DMA((NK,)),
            pltpu.SemaphoreType.DMA((9,)),
        ],
        compiler_params=pltpu.CompilerParams(vmem_limit_bytes=100 * 1024 * 1024),
    )(*ins).reshape(B, Sq, D)
```
